```python
import jax
import jax.numpy as jnp

def _softmax(x, axis=-1):
    return jax.nn.softmax(x, axis=axis)
def _gelu(x):
    return jax.nn.gelu(x, approximate=True)
def _silu(x):
    return jax.nn.silu(x)
def _sigmoid(x):
    return jax.nn.sigmoid(x)
def _layernorm(x, axis=-1, eps=1e-5):
    m = jnp.mean(x, axis=axis, keepdims=True)
    v = jnp.var(x, axis=axis, keepdims=True)
    return (x - m) / jnp.sqrt(v + eps)
def _scatter_add(tgt, idx, src, axis=0):
    return tgt.at[idx].add(src)
def _segment_sum(src, seg, n):
    return jax.ops.segment_sum(src, seg, n)
class _Rng:
    def __init__(self, key):
        self._k = key
    def _next(self):
        self._k, sub = jax.random.split(self._k)
        return sub
    def normal(self, shape):
        return jax.random.normal(self._next(), shape, dtype=jnp.bfloat16)
    def randint(self, lo, hi, shape):
        return jax.random.randint(self._next(), shape, lo, hi, dtype=jnp.int32)
    def uniform(self, shape, lo=0.0, hi=1.0):
        return jax.random.uniform(self._next(), shape, jnp.bfloat16, lo, hi)
    def permutation(self, n):
        return jax.random.permutation(self._next(), n)


kernel_name = 'standalone__structured_sparse_n_m__ragged'

def setup_inputs():
    _rng = _Rng(jax.random.key(int.from_bytes(__import__("os").urandom(4), "little")))
    _w = (lambda a: (lambda t: t.astype(jnp.bfloat16) if jnp.issubdtype(t.dtype, jnp.floating) else t)(jnp.asarray(a)))
    B, S, D = 16, 4096, 576
    assert D % 4 == 0, "d_model must be divisible by M=4 for 2:4 sparsity"
    return {
        "x": _w((lambda *s: _rng.normal(s) * 0.05)(B, S, D)),
        "w": _w((lambda *s: _rng.normal(s) * 0.05)(D, D)),
        "b": _w((lambda *s: _rng.normal(s) * 0.05)(D)),
    }

def reference(x, w, b):
    B, S, D = x.shape
    N, M = 2, 4
    G = D // M
    wg = w.reshape(G, M, D)
    mag = jnp.abs(wg)
    order = jnp.argsort(mag, 1)
    thr = jnp.take_along_axis(mag, order[:, M - N:M - N + 1, :], 1)
    mask = (lambda x, dt: x.astype(dt))(mag >= thr, w.dtype)
    wp = (wg * mask).reshape(D, D)
    return jnp.einsum("bsd,df->bsf", x, wp) + b
```

```python
import jax
import jax.numpy as jnp
from jax import lax
import jax.experimental.pallas as pl
import jax.experimental.pallas.tpu as pltpu

_KPAD = 64


def _prune_packed(u):
    even = (lax.broadcasted_iota(jnp.int32, u.shape, 0) & 1) == 0
    lo = pltpu.bitcast((u << 16) & 0x7FFFFFFF, jnp.float32)
    hi = pltpu.bitcast(u & 0x7FFF0000, jnp.float32)
    nlo = jnp.where(even, pltpu.roll(lo, 7, 0), pltpu.roll(lo, 1, 0))
    nhi = jnp.where(even, pltpu.roll(hi, 7, 0), pltpu.roll(hi, 1, 0))
    thr = jnp.maximum(
        jnp.minimum(jnp.maximum(lo, hi), jnp.maximum(nlo, nhi)),
        jnp.maximum(jnp.minimum(lo, hi), jnp.minimum(nlo, nhi)),
    )
    return u & (jnp.where(lo < thr, 0, 0xFFFF) | jnp.where(hi < thr, 0, -65536))


def _prepare_weights(w_ref, b_ref, wt_ref):
    d, f = w_ref.shape
    u = pltpu.bitcast(w_ref[...], jnp.int32)
    parts = [_prune_packed(u[8 * i:8 * i + 8]) for i in range(d // 16)]
    bias = b_ref[...].reshape(1, f).astype(jnp.float32)
    bits = (pltpu.bitcast(bias, jnp.int32) >> 16) & 0xFFFF
    row = lax.broadcasted_iota(jnp.int32, (_KPAD // 2, f), 0)
    parts.append(jnp.where(row == 0, jnp.broadcast_to(bits, (_KPAD // 2, f)), 0))
    wp = pltpu.bitcast(jnp.concatenate(parts, axis=0), jnp.bfloat16)
    wt_ref[...] = pltpu.bitcast(wp.T, jnp.int32)


HEAD = (512, 512, 1024, 2048)
TAIL = (2048, 1024, 512, 512)
NX = 2
NO = 2


def _kernel(x_hbm, w_hbm, b_hbm, o_hbm, xbuf, obuf, wbuf, bbuf, wt_ref,
            wsem, hsem, xsem, osem):
    NB, _, S = x_hbm.shape
    hoff = [sum(HEAD[:j]) for j in range(len(HEAD))]
    toff = [sum(TAIL[:j]) for j in range(len(TAIL))]
    wcp = pltpu.make_async_copy(w_hbm, wbuf, wsem.at[0])
    bcp = pltpu.make_async_copy(b_hbm, bbuf, wsem.at[1])

    def hcopy(j):
        sl = pl.ds(hoff[j], HEAD[j])
        return pltpu.make_async_copy(x_hbm.at[0, :, sl], xbuf.at[0, :, sl], hsem.at[j])

    def xcopy(i):
        return pltpu.make_async_copy(x_hbm.at[i], xbuf.at[i % NX], xsem.at[i % NX])

    def opart(i, off, n):
        sl = pl.ds(off, n)
        return pltpu.make_async_copy(
            obuf.at[i % NO, :, sl], o_hbm.at[i, :, sl], osem.at[i % NO])

    def ocopy(i):
        return pltpu.make_async_copy(obuf.at[i % NO], o_hbm.at[i], osem.at[i % NO])

    def compute(xs, os_, off, n):
        wt = pltpu.bitcast(wt_ref[...], jnp.bfloat16)
        row = lax.broadcasted_iota(jnp.int32, (_KPAD, n), 0)
        ones = jnp.where(row == 0, 1.0, 0.0).astype(jnp.bfloat16)
        rhs = jnp.concatenate([xbuf[xs, :, pl.ds(off, n)], ones], axis=0)
        obuf[os_, :, pl.ds(off, n)] = jnp.dot(
            wt, rhs, preferred_element_type=jnp.float32).astype(jnp.bfloat16)

    wcp.start()
    bcp.start()
    hcopy(0).start()
    hcopy(1).start()
    wcp.wait()
    bcp.wait()
    _prepare_weights(wbuf, bbuf, wt_ref)
    nh = len(HEAD)
    nxt = 1
    for j in range(nh):
        hcopy(j).wait()
        if j + 2 < nh:
            hcopy(j + 2).start()
        elif nxt < NX:
            xcopy(nxt).start()
            nxt += 1
        compute(0, 0, hoff[j], HEAD[j])
        opart(0, hoff[j], HEAD[j]).start()
    while nxt < NX:
        xcopy(nxt).start()
        nxt += 1

    def body(i, c):
        xcopy(i).wait()

        @pl.when(i >= NO)
        def _():
            ocopy(i - NO).wait()

        @pl.when(i + NX - 1 < NB)
        def _():
            xcopy(i + NX - 1).start()

        compute(i % NX, i % NO, 0, S)
        ocopy(i).start()
        return c

    lax.fori_loop(1, NB - 1, body, 0)
    i = NB - 1
    xcopy(i).wait()
    ocopy(i - NO).wait()
    for j in range(len(TAIL)):
        compute(i % NX, i % NO, toff[j], TAIL[j])
        opart(i, toff[j], TAIL[j]).start()
    for k in range(i - NO + 1, i + 1):
        ocopy(k).wait()


@jax.jit
def pallas_standalone__structured_sparse_n_m__ragged_kernel(
    x: jax.Array,
    w: jax.Array,
    b: jax.Array,
):
    B, S, D = x.shape
    F = w.shape[1]
    xt = jnp.transpose(x, (0, 2, 1))
    out = pl.pallas_call(
        _kernel,
        in_specs=[pl.BlockSpec(memory_space=pl.ANY)] * 3,
        out_specs=pl.BlockSpec(memory_space=pl.ANY),
        out_shape=jax.ShapeDtypeStruct((B, F, S), x.dtype),
        scratch_shapes=[
            pltpu.VMEM((NX, D, S), x.dtype),
            pltpu.VMEM((NO, F, S), x.dtype),
            pltpu.VMEM((D, F), w.dtype),
            pltpu.VMEM((F,), b.dtype),
            pltpu.VMEM((F // 2, D + _KPAD), jnp.int32),
            pltpu.SemaphoreType.DMA((2,)),
            pltpu.SemaphoreType.DMA((len(HEAD),)),
            pltpu.SemaphoreType.DMA((NX,)),
            pltpu.SemaphoreType.DMA((NO,)),
        ],
        compiler_params=pltpu.CompilerParams(vmem_limit_bytes=100 * 1024 * 1024),
    )(xt, w, b)
    return jnp.transpose(out, (0, 2, 1))
```

```python
import jax
import jax.numpy as jnp
from jax import lax
import jax.experimental.pallas as pl
import jax.experimental.pallas.tpu as pltpu

_KM = 512
_KPAD = 64

R = 80
NPAIR = 12
LANES = 2
U = 2
IN_FIRST = (512, 512, 1024, 2048)
OUT_LAST = (2048, 1024, 512, 256, 128, 128)


def _prune_packed(u):
    even = (lax.broadcasted_iota(jnp.int32, u.shape, 0) & 1) == 0
    lo = pltpu.bitcast((u << 16) & 0x7FFFFFFF, jnp.float32)
    hi = pltpu.bitcast(u & 0x7FFF0000, jnp.float32)
    nlo = jnp.where(even, pltpu.roll(lo, 7, 0), pltpu.roll(lo, 1, 0))
    nhi = jnp.where(even, pltpu.roll(hi, 7, 0), pltpu.roll(hi, 1, 0))
    thr = jnp.maximum(
        jnp.minimum(jnp.maximum(lo, hi), jnp.maximum(nlo, nhi)),
        jnp.maximum(jnp.minimum(lo, hi), jnp.minimum(nlo, nhi)),
    )
    return u & (jnp.where(lo < thr, 0, 0xFFFF) | jnp.where(hi < thr, 0, -65536))


def _prune_rows(w_bf16):
    u = pltpu.bitcast(w_bf16, jnp.int32)
    return [_prune_packed(u[8 * i:8 * i + 8]) for i in range(u.shape[0] // 8)]


def _split(total, sizes):
    assert sum(sizes) == total
    return [(sum(sizes[:j]), sizes[j]) for j in range(len(sizes))]


def _kernel(x_hbm, w_hbm, b_hbm, o_hbm, xbuf, obuf, wbuf, bbuf, wt_ref, wb_ref, isem, osem):
    NB, D, S = x_hbm.shape
    F = w_hbm.shape[1]
    KT = D - _KM
    NIT = NB // U
    in_chunks = [(0, o, n) for o, n in _split(S, IN_FIRST)] + [(u, 0, S) for u in range(1, U)]
    out_chunks = [(u, 0, S) for u in range(U - 1)] + [(U - 1, o, n) for o, n in _split(S, OUT_LAST)]
    ni = len(in_chunks)

    def icopy(t, j):
        u, o, n = in_chunks[j]
        return pltpu.make_async_copy(
            x_hbm.at[t * U + u, :, pl.ds(o, n)], xbuf.at[u, :, pl.ds(o, n)], isem.at[j])

    def ocopy(t, j):
        u, o, n = out_chunks[j]
        return pltpu.make_async_copy(
            obuf.at[u, :, pl.ds(o, n)], o_hbm.at[t * U + u, :, pl.ds(o, n)], osem.at[j])

    bcp = pltpu.make_async_copy(b_hbm, bbuf, isem.at[ni])
    wtail = pltpu.make_async_copy(
        w_hbm.at[pl.ds(_KM, KT)], wbuf.at[pl.ds(_KM, KT)], isem.at[ni + 1])
    wmain = pltpu.make_async_copy(
        w_hbm.at[pl.ds(0, _KM)], wbuf.at[pl.ds(0, _KM)], isem.at[ni + 2])
    bcp.start()
    wtail.start()
    wmain.start()
    bcp.wait()
    for j in range(ni):
        icopy(0, j).start()

    wtail.wait()
    parts = _prune_rows(wbuf[_KM:D, :])
    bias = bbuf[...].reshape(1, F).astype(jnp.float32)
    bits = (pltpu.bitcast(bias, jnp.int32) >> 16) & 0xFFFF
    row = lax.broadcasted_iota(jnp.int32, (_KPAD // 2, F), 0)
    parts.append(jnp.where(row == 0, jnp.broadcast_to(bits, (_KPAD // 2, F)), 0))
    wt_tail = pltpu.bitcast(jnp.concatenate(parts, axis=0), jnp.bfloat16).T
    wt_ref[:, _KM:] = pltpu.bitcast(wt_tail, jnp.int32)
    w_vpu = wt_tail[0:R].astype(jnp.float32)
    for k in range(KT + 1):
        wb_ref[k] = jnp.broadcast_to(w_vpu[:, k:k + 1], (R, 128))
    wb_ref[KT + 1] = jnp.zeros((R, 128), jnp.float32)

    wmain.wait()
    parts = _prune_rows(wbuf[0:_KM, :])
    wp = pltpu.bitcast(jnp.concatenate(parts, axis=0), jnp.bfloat16)
    wt_ref[:, 0:_KM] = pltpu.bitcast(wp.T, jnp.int32)

    xwords = xbuf.bitcast(jnp.int32)

    def tail_on_vpu(u, o, n, acc_main, state):
        always, prev = state
        cols = []
        for t0 in range(0, n, 128):
            rows = []
            for f0 in range(0, R // 8, LANES):
                ids = range(min(LANES, R // 8 - f0))
                sl = [pl.ds((f0 + a) * 8, 8) for a in ids]
                acc = []
                for a in ids:
                    v = wb_ref[KT, sl[a], :]
                    acc.append(jnp.where(always, v, prev[a]) if a in prev else v)

                def prod(k):
                    q = jnp.broadcast_to(
                        xwords[u, pl.ds((_KM + k) // 2, 1), pl.ds(o + t0, 128)], (8, 128))
                    xk = pltpu.bitcast((q << 16) if k % 2 == 0 else (q & -65536), jnp.float32)
                    return [wb_ref[k, sl[a], :] * xk for a in ids]

                steps = KT - NPAIR
                k = 0
                for st in range(steps):
                    p = prod(k)
                    k += 1
                    if (st * NPAIR) // steps != ((st + 1) * NPAIR) // steps:
                        p2 = prod(k)
                        k += 1
                        p = [p[a] + p2[a] for a in ids]
                    acc = [acc[a] + p[a] for a in ids]
                assert k == KT
                for a in ids:
                    prev[a] = acc[a]
                    rows.append(acc[a] + acc_main[(f0 + a) * 8:(f0 + a + 1) * 8, t0:t0 + 128])
            cols.append(jnp.concatenate(rows, axis=0))
        return jnp.concatenate(cols, axis=1)

    def compute(u, o, n, state):
        row = lax.broadcasted_iota(jnp.int32, (_KPAD, n), 0)
        ones = jnp.where(row == 0, 1.0, 0.0).astype(jnp.bfloat16)
        xx = xbuf[u, :, pl.ds(o, n)]
        x_tail = jnp.concatenate([xx[_KM:], ones], axis=0)
        acc_main = jnp.dot(pltpu.bitcast(wt_ref[:, 0:_KM], jnp.bfloat16), xx[:_KM],
                           preferred_element_type=jnp.float32)
        acc_tail = jnp.dot(pltpu.bitcast(wt_ref[R // 2:, _KM:], jnp.bfloat16), x_tail,
                           preferred_element_type=jnp.float32)
        obuf[u, R:, pl.ds(o, n)] = (acc_main[R:] + acc_tail).astype(obuf.dtype)
        obuf[u, 0:R, pl.ds(o, n)] = tail_on_vpu(u, o, n, acc_main, state).astype(obuf.dtype)

    def body(t, carry):
        state = (wb_ref[KT + 1, 0:8, :] == 0.0, {})
        for u in range(U):
            ins = [(j, o, n) for j, (uu, o, n) in enumerate(in_chunks) if uu == u]
            outs = [(j, o, n) for j, (uu, o, n) in enumerate(out_chunks) if uu == u]
            pts = sorted({S} | {o for _, o, _ in ins + outs})
            for lo, hi in zip(pts[:-1], pts[1:]):
                for j, o, n in ins:
                    if o == lo:
                        icopy(t, j).wait()
                for j, o, n in outs:
                    if o == lo:
                        @pl.when(t > 0)
                        def _():
                            ocopy(t - 1, j).wait()
                compute(u, lo, hi - lo, state)
                for j, o, n in ins:
                    if o + n == hi:
                        @pl.when(t + 1 < NIT)
                        def _():
                            icopy(t + 1, j).start()
                for j, o, n in outs:
                    if o + n == hi:
                        ocopy(t, j).start()
        return carry

    lax.fori_loop(0, NIT, body, 0)
    for j in range(len(out_chunks)):
        ocopy(NIT - 1, j).wait()


@jax.jit
def pallas_standalone__structured_sparse_n_m__ragged_kernel(
    x: jax.Array,
    w: jax.Array,
    b: jax.Array,
):
    B, S, D = x.shape
    F = w.shape[1]
    xt = jnp.transpose(x, (0, 2, 1))
    n_in = len(IN_FIRST) + U - 1
    n_out = len(OUT_LAST) + U - 1
    out = pl.pallas_call(
        _kernel,
        in_specs=[pl.BlockSpec(memory_space=pl.ANY)] * 3,
        out_specs=pl.BlockSpec(memory_space=pl.ANY),
        out_shape=jax.ShapeDtypeStruct((B, F, S), x.dtype),
        scratch_shapes=[
            pltpu.VMEM((U, D, S), x.dtype),
            pltpu.VMEM((U, F, S), x.dtype),
            pltpu.VMEM((D, F), w.dtype),
            pltpu.VMEM((F,), b.dtype),
            pltpu.VMEM((F // 2, D + _KPAD), jnp.int32),
            pltpu.VMEM((D - _KM + 2, R, 128), jnp.float32),
            pltpu.SemaphoreType.DMA((n_in + 3,)),
            pltpu.SemaphoreType.DMA((n_out,)),
        ],
        compiler_params=pltpu.CompilerParams(
            vmem_limit_bytes=100 * 1024 * 1024,
            flags={"XLA_TPU_RESCHEDULE_DMA_DONES": True},
        ),
    )(xt, w, b)
    return jnp.transpose(out, (0, 2, 1))
```

```python
import jax
import jax.numpy as jnp
from jax import lax
import jax.experimental.pallas as pl
import jax.experimental.pallas.tpu as pltpu

_KM = 512
_KPAD = 64

R = 80
R_FIRST = 64
GROUP = 512
LANES = 2
U = 2
IN_FIRST = (256, 256, 512, 1024, 2048)
OUT_LAST = (2048, 1024, 512, 256, 128, 128)


def _prune_packed(u):
    mate = lax.broadcasted_iota(jnp.int32, u.shape, 0) ^ 1
    lo = pltpu.bitcast((u << 16) & 0x7FFFFFFF, jnp.float32)
    hi = pltpu.bitcast(u & 0x7FFF0000, jnp.float32)
    big, small = jnp.maximum(lo, hi), jnp.minimum(lo, hi)
    nbig = jnp.take_along_axis(big, mate, axis=0, mode="promise_in_bounds")
    nsmall = jnp.take_along_axis(small, mate, axis=0, mode="promise_in_bounds")
    thr = jnp.maximum(jnp.minimum(big, nbig), jnp.maximum(small, nsmall))
    return u & (jnp.where(lo < thr, 0, 0xFFFF) | jnp.where(hi < thr, 0, -65536))


def _prune_rows(w_bf16):
    u = pltpu.bitcast(w_bf16, jnp.int32)
    return [_prune_packed(u[8 * i:8 * i + 8]) for i in range(u.shape[0] // 8)]


def _split(total, sizes):
    assert sum(sizes) == total
    return [(sum(sizes[:j]), sizes[j]) for j in range(len(sizes))]


def _kernel(x_hbm, w_hbm, b_hbm, o_hbm, xbuf, obuf, wbuf, bbuf, wt_ref, wb_ref, isem, osem):
    NB, D, S = x_hbm.shape
    F = w_hbm.shape[1]
    KT = D - _KM
    NIT = NB // U
    in_chunks = [(0, o, n) for o, n in _split(S, IN_FIRST)] + [(u, 0, S) for u in range(1, U)]
    out_chunks = [(u, 0, S) for u in range(U - 1)] + [(U - 1, o, n) for o, n in _split(S, OUT_LAST)]
    ni = len(in_chunks)

    def icopy(t, j):
        u, o, n = in_chunks[j]
        return pltpu.make_async_copy(
            x_hbm.at[t * U + u, :, pl.ds(o, n)], xbuf.at[u, :, pl.ds(o, n)], isem.at[j])

    def ocopy(t, j):
        u, o, n = out_chunks[j]
        return pltpu.make_async_copy(
            obuf.at[u, :, pl.ds(o, n)], o_hbm.at[t * U + u, :, pl.ds(o, n)], osem.at[j])

    bcp = pltpu.make_async_copy(b_hbm, bbuf, isem.at[ni])
    wtail = pltpu.make_async_copy(
        w_hbm.at[pl.ds(_KM, KT)], wbuf.at[pl.ds(_KM, KT)], isem.at[ni + 1])
    wmain = pltpu.make_async_copy(
        w_hbm.at[pl.ds(0, _KM)], wbuf.at[pl.ds(0, _KM)], isem.at[ni + 2])
    bcp.start()
    wtail.start()
    wmain.start()
    bcp.wait()
    for j in range(ni):
        icopy(0, j).start()

    wtail.wait()
    parts = _prune_rows(wbuf[_KM:D, :])
    bias = bbuf[...].reshape(1, F).astype(jnp.float32)
    bits = (pltpu.bitcast(bias, jnp.int32) >> 16) & 0xFFFF
    row = lax.broadcasted_iota(jnp.int32, (_KPAD // 2, F), 0)
    parts.append(jnp.where(row == 0, jnp.broadcast_to(bits, (_KPAD // 2, F)), 0))
    wt_tail = pltpu.bitcast(jnp.concatenate(parts, axis=0), jnp.bfloat16).T
    wt_ref[:, _KM:] = pltpu.bitcast(wt_tail, jnp.int32)
    w_vpu = wt_tail[0:R].astype(jnp.float32)
    for k in range(KT + 1):
        wb_ref[k] = jnp.broadcast_to(w_vpu[:, k:k + 1], (R, 128))
    wb_ref[KT + 1] = jnp.zeros((R, 128), jnp.float32)

    wmain.wait()
    parts = _prune_rows(wbuf[0:_KM, :])
    wp = pltpu.bitcast(jnp.concatenate(parts, axis=0), jnp.bfloat16)
    wt_ref[:, 0:_KM] = pltpu.bitcast(wp.T, jnp.int32)

    xwords = xbuf.bitcast(jnp.int32)

    def tail_on_vpu(u, o, n, r, acc_main, state):
        always, prev = state
        cols = []
        for t0 in range(0, n, 128):
            rows = []
            for f0 in range(0, r // 8, LANES):
                ids = range(min(LANES, r // 8 - f0))
                sl = [pl.ds((f0 + a) * 8, 8) for a in ids]
                acc = []
                for a in ids:
                    v = wb_ref[KT, sl[a], :]
                    acc.append(jnp.where(always, v, prev[a]) if a in prev else v)

                for k in range(KT):
                    q = jnp.broadcast_to(
                        xwords[u, pl.ds((_KM + k) // 2, 1), pl.ds(o + t0, 128)], (8, 128))
                    xk = pltpu.bitcast((q << 16) if k % 2 == 0 else (q & -65536), jnp.float32)
                    acc = [acc[a] + wb_ref[k, sl[a], :] * xk for a in ids]
                for a in ids:
                    prev[a] = acc[a]
                    rows.append(acc[a] + acc_main[(f0 + a) * 8:(f0 + a + 1) * 8, t0:t0 + 128])
            cols.append(jnp.concatenate(rows, axis=0))
        return jnp.concatenate(cols, axis=1)

    def compute(u, o, n, state):
        r = R_FIRST if u == 0 and o < GROUP else R
        row = lax.broadcasted_iota(jnp.int32, (_KPAD, n), 0)
        ones = jnp.where(row == 0, 1.0, 0.0).astype(jnp.bfloat16)
        xx = xbuf[u, :, pl.ds(o, n)]
        x_tail = jnp.concatenate([xx[_KM:], ones], axis=0)
        acc_main = jnp.dot(pltpu.bitcast(wt_ref[:, 0:_KM], jnp.bfloat16), xx[:_KM],
                           preferred_element_type=jnp.float32)
        acc_tail = jnp.dot(pltpu.bitcast(wt_ref[r // 2:, _KM:], jnp.bfloat16), x_tail,
                           preferred_element_type=jnp.float32)
        obuf[u, r:, pl.ds(o, n)] = (acc_main[r:] + acc_tail).astype(obuf.dtype)
        obuf[u, 0:r, pl.ds(o, n)] = tail_on_vpu(u, o, n, r, acc_main, state).astype(obuf.dtype)

    def body(t, carry):
        state = (wb_ref[KT + 1, 0:8, :] == 0.0, {})
        for u in range(U):
            ins = [(j, o, n) for j, (uu, o, n) in enumerate(in_chunks) if uu == u]
            outs = [(j, o, n) for j, (uu, o, n) in enumerate(out_chunks) if uu == u]
            pts = sorted(set(range(0, S + 1, GROUP)) | {o for _, o, _ in ins + outs})
            for lo, hi in zip(pts[:-1], pts[1:]):
                for j, o, n in ins:
                    if o == lo:
                        icopy(t, j).wait()
                for j, o, n in outs:
                    if o == lo:
                        @pl.when(t > 0)
                        def _():
                            ocopy(t - 1, j).wait()
                compute(u, lo, hi - lo, state)
                for j, o, n in ins:
                    if o + n == hi:
                        @pl.when(t + 1 < NIT)
                        def _():
                            icopy(t + 1, j).start()
                for j, o, n in outs:
                    if o + n == hi:
                        ocopy(t, j).start()
        return carry

    lax.fori_loop(0, NIT, body, 0)
    for j in range(len(out_chunks)):
        ocopy(NIT - 1, j).wait()


@jax.jit
def pallas_standalone__structured_sparse_n_m__ragged_kernel(
    x: jax.Array,
    w: jax.Array,
    b: jax.Array,
):
    B, S, D = x.shape
    F = w.shape[1]
    xt = jnp.transpose(x, (0, 2, 1))
    n_in = len(IN_FIRST) + U - 1
    n_out = len(OUT_LAST) + U - 1
    out = pl.pallas_call(
        _kernel,
        in_specs=[pl.BlockSpec(memory_space=pl.ANY)] * 3,
        out_specs=pl.BlockSpec(memory_space=pl.ANY),
        out_shape=jax.ShapeDtypeStruct((B, F, S), x.dtype),
        scratch_shapes=[
            pltpu.VMEM((U, D, S), x.dtype),
            pltpu.VMEM((U, F, S), x.dtype),
            pltpu.VMEM((D, F), w.dtype),
            pltpu.VMEM((F,), b.dtype),
            pltpu.VMEM((F // 2, D + _KPAD), jnp.int32),
            pltpu.VMEM((D - _KM + 2, R, 128), jnp.float32),
            pltpu.SemaphoreType.DMA((n_in + 3,)),
            pltpu.SemaphoreType.DMA((n_out,)),
        ],
        compiler_params=pltpu.CompilerParams(
            vmem_limit_bytes=100 * 1024 * 1024,
            flags={"XLA_TPU_RESCHEDULE_DMA_DONES": True},
        ),
    )(xt, w, b)
    return jnp.transpose(out, (0, 2, 1))
```
